```python
import os as _os
_os.environ.setdefault("JAX_PLATFORMS", "cpu")
import jax
import jax.numpy as jnp

def _softmax(x, axis=-1):
    return jax.nn.softmax(x, axis=axis)
def _gelu(x):
    return jax.nn.gelu(x, approximate=True)
def _silu(x):
    return jax.nn.silu(x)
def _sigmoid(x):
    return jax.nn.sigmoid(x)
def _layernorm(x, axis=-1, eps=1e-5):
    m = jnp.mean(x, axis=axis, keepdims=True)
    v = jnp.var(x, axis=axis, keepdims=True)
    return (x - m) / jnp.sqrt(v + eps)
def _scatter_add(tgt, idx, src, axis=0):
    return tgt.at[idx].add(src)
def _segment_sum(src, seg, n):
    return jax.ops.segment_sum(src, seg, n)
class _Rng:
    def __init__(self, key):
        self._k = key
    def _next(self):
        self._k, sub = jax.random.split(self._k)
        return sub
    def normal(self, shape):
        return jax.random.normal(self._next(), shape, dtype=jnp.bfloat16)
    def randint(self, lo, hi, shape):
        return jax.random.randint(self._next(), shape, lo, hi, dtype=jnp.int32)
    def uniform(self, shape, lo=0.0, hi=1.0):
        return jax.random.uniform(self._next(), shape, jnp.bfloat16, lo, hi)
    def permutation(self, n):
        return jax.random.permutation(self._next(), n)


kernel_name = 'concat_heads__mha_block_cached__mha_block_cached__near_ridge'

def setup_inputs():
    _rng = _Rng(jax.random.key(int.from_bytes(__import__("os").urandom(4), "little")))
    _w = (lambda a: (lambda t: t.astype(jnp.bfloat16) if jnp.issubdtype(t.dtype, jnp.floating) else t)(jnp.asarray(a)))
    def _A_setup():
        B, Sq, D = 8, 160, 512
        H, Sk, Dh = 32, 512, 128
        return {
            "x": _w((lambda *s: _rng.normal(s) * 0.8)(B, Sq, D)),
            "k_cache": _w((lambda *s: _rng.normal(s) * 0.8)(B, H, Sk, Dh)),
            "v_cache": _w((lambda *s: _rng.normal(s) * 0.05)(B, H, Sk, Dh)),
            "wq": _w((lambda *s: _rng.normal(s) * 0.8)(D, H * Dh) * (D ** -0.5)),
            "wo": _w((lambda *s: _rng.normal(s) * 0.05)(H * Dh, D) * ((H * Dh) ** -0.5)),
        }
    _A_in = _A_setup()

    def _B_setup():
        B, Sq, D = 8, 160, 512
        H, Sk, Dh = 32, 512, 128
        return {
            "x": _w((lambda *s: _rng.normal(s) * 0.8)(B, Sq, D)),
            "k_cache": _w((lambda *s: _rng.normal(s) * 0.8)(B, H, Sk, Dh)),
            "v_cache": _w((lambda *s: _rng.normal(s) * 0.05)(B, H, Sk, Dh)),
            "wq": _w((lambda *s: _rng.normal(s) * 0.8)(D, H * Dh) * (D ** -0.5)),
            "wo": _w((lambda *s: _rng.normal(s) * 0.05)(H * Dh, D) * ((H * Dh) ** -0.5)),
        }
    _B_in = _B_setup()

    return {
        "A_x": _A_in["x"],
        "A_k_cache": _A_in["k_cache"],
        "A_v_cache": _A_in["v_cache"],
        "A_wq": _A_in["wq"],
        "A_wo": _A_in["wo"],
        "B_x": _B_in["x"],
        "B_k_cache": _B_in["k_cache"],
        "B_v_cache": _B_in["v_cache"],
        "B_wq": _B_in["wq"],
        "B_wo": _B_in["wo"],
    }

def reference(A_x, A_k_cache, A_v_cache, A_wq, A_wo, B_x, B_k_cache, B_v_cache, B_wq, B_wo):
    def _A_ref(x, k_cache, v_cache, wq, wo):
        B, Sq, D = x.shape
        H, Dh = 32, 128
        q = (lambda x, *d: x.transpose(*d))((x @ wq).reshape(B, Sq, H, Dh), 0, 2, 1, 3)
        scores = jnp.einsum("bhqd,bhkd->bhqk", q, k_cache) * (Dh ** -0.5)
        p = _softmax(scores, axis=-1)
        o = jnp.einsum("bhqk,bhkd->bhqd", p, v_cache)
        return (lambda x, *d: x.transpose(*d))(o, 0, 2, 1, 3).reshape(B, Sq, H * Dh) @ wo

    def _B_ref(x, k_cache, v_cache, wq, wo):
        B, Sq, D = x.shape
        H, Dh = 32, 128
        q = (lambda x, *d: x.transpose(*d))((x @ wq).reshape(B, Sq, H, Dh), 0, 2, 1, 3)
        scores = jnp.einsum("bhqd,bhkd->bhqk", q, k_cache) * (Dh ** -0.5)
        p = _softmax(scores, axis=-1)
        o = jnp.einsum("bhqk,bhkd->bhqd", p, v_cache)
        return (lambda x, *d: x.transpose(*d))(o, 0, 2, 1, 3).reshape(B, Sq, H * Dh) @ wo

    a = _A_ref(A_x, A_k_cache, A_v_cache, A_wq, A_wo)
    b = _B_ref(B_x, B_k_cache, B_v_cache, B_wq, B_wo)
    return jnp.concatenate([a, b], axis=-1)
```

```python
import functools

import jax
import jax.numpy as jnp
from jax import lax
import jax.experimental.pallas as pl
import jax.experimental.pallas.tpu as pltpu


def _attn_block(x, wq, wo, k_ref, v_ref, G, Dh):
    scale = Dh ** -0.5
    q = jnp.dot(x, wq, preferred_element_type=jnp.float32) * scale
    q = q.astype(jnp.bfloat16)
    outs = []
    for h in range(G):
        qh = q[:, h * Dh:(h + 1) * Dh]
        kh = k_ref[0, h]
        vh = v_ref[0, h]
        s = lax.dot_general(qh, kh, (((1,), (1,)), ((), ())),
                            preferred_element_type=jnp.float32)
        m = jnp.max(s, axis=-1, keepdims=True)
        p = jnp.exp(s - m)
        l = jnp.sum(p, axis=-1, keepdims=True)
        o = jnp.dot(p.astype(jnp.bfloat16), vh,
                    preferred_element_type=jnp.float32)
        o = o * pl.reciprocal(l, approx=False)
        outs.append(o.astype(jnp.bfloat16))
    o_all = jnp.concatenate(outs, axis=-1)
    return jnp.dot(o_all, wo, preferred_element_type=jnp.float32)


def _kernel(ax_ref, ak_ref, av_ref, awq_ref, awo_ref,
            bx_ref, bk_ref, bv_ref, bwq_ref, bwo_ref,
            o_ref, acc_ref, *, G, Dh, D):
    hg = pl.program_id(0)
    b = pl.program_id(1)
    n_hg = pl.num_programs(0)

    ya = _attn_block(ax_ref[b], awq_ref[...], awo_ref[...], ak_ref, av_ref, G, Dh)
    yb = _attn_block(bx_ref[b], bwq_ref[...], bwo_ref[...], bk_ref, bv_ref, G, Dh)

    @pl.when(hg == 0)
    def _():
        acc_ref[b, :, 0:D] = ya
        acc_ref[b, :, D:2 * D] = yb

    @pl.when(hg > 0)
    def _():
        acc_ref[b, :, 0:D] += ya
        acc_ref[b, :, D:2 * D] += yb

    @pl.when(hg == n_hg - 1)
    def _():
        o_ref[b] = acc_ref[b].astype(o_ref.dtype)


@jax.jit
def pallas_concat_heads__mha_block_cached__mha_block_cached__near_ridge_kernel(
    A_x: jax.Array,
    A_k_cache: jax.Array,
    A_v_cache: jax.Array,
    A_wq: jax.Array,
    A_wo: jax.Array,
    B_x: jax.Array,
    B_k_cache: jax.Array,
    B_v_cache: jax.Array,
    B_wq: jax.Array,
    B_wo: jax.Array,
):
    B, Sq, D = A_x.shape
    _, H, Sk, Dh = A_k_cache.shape
    G = 8
    n_hg = H // G

    x_spec = pl.BlockSpec((B, Sq, D), lambda hg, b: (0, 0, 0))
    kv_spec = pl.BlockSpec((1, G, Sk, Dh), lambda hg, b: (b, hg, 0, 0))
    wq_spec = pl.BlockSpec((D, G * Dh), lambda hg, b: (0, hg))
    wo_spec = pl.BlockSpec((G * Dh, D), lambda hg, b: (hg, 0))
    out_spec = pl.BlockSpec((B, Sq, 2 * D), lambda hg, b: (0, 0, 0))

    kernel = functools.partial(_kernel, G=G, Dh=Dh, D=D)
    return pl.pallas_call(
        kernel,
        grid=(n_hg, B),
        in_specs=[x_spec, kv_spec, kv_spec, wq_spec, wo_spec,
                  x_spec, kv_spec, kv_spec, wq_spec, wo_spec],
        out_specs=out_spec,
        out_shape=jax.ShapeDtypeStruct((B, Sq, 2 * D), A_x.dtype),
        scratch_shapes=[pltpu.VMEM((B, Sq, 2 * D), jnp.float32)],
        compiler_params=pltpu.CompilerParams(
            dimension_semantics=("arbitrary", "arbitrary"),
            vmem_limit_bytes=100 * 1024 * 1024,
        ),
    )(A_x, A_k_cache, A_v_cache, A_wq, A_wo,
      B_x, B_k_cache, B_v_cache, B_wq, B_wo)
```

```python
import functools

import jax
import jax.numpy as jnp
from jax import lax
import jax.experimental.pallas as pl
import jax.experimental.pallas.tpu as pltpu


def _kernel(ax_hbm, ak_hbm, av_hbm, awq_hbm, awo_hbm,
            bx_hbm, bk_hbm, bv_hbm, bwq_hbm, bwo_hbm,
            o_ref,
            x_buf, k_buf, v_buf, wq_buf, wo_buf, acc_ref,
            x_sem, kv_sem, w_sem, *, G, Dh, D, NB, NHG):
    hg = pl.program_id(0)
    b = pl.program_id(1)
    step = hg * NB + b
    n_steps = NHG * NB
    slot = lax.rem(step, 2)
    wslot = lax.rem(hg, 2)
    scale = Dh ** -0.5
    GD = G * Dh

    x_hbm = (ax_hbm, bx_hbm)
    k_hbm = (ak_hbm, bk_hbm)
    v_hbm = (av_hbm, bv_hbm)
    wq_hbm = (awq_hbm, bwq_hbm)
    wo_hbm = (awo_hbm, bwo_hbm)

    units = [(c, h) for c in range(2) for h in range(G)]
    n = len(units)

    def x_copy(c, b_):
        return pltpu.make_async_copy(x_hbm[c].at[b_], x_buf.at[c, b_],
                                     x_sem.at[lax.rem(b_, 2) * 2 + c])

    def k_copy(c, hg_, b_, slot_):
        return pltpu.make_async_copy(k_hbm[c].at[b_, pl.ds(hg_ * G, G)],
                                     k_buf.at[slot_, c],
                                     kv_sem.at[slot_ * 4 + c * 2])

    def v_copy(c, hg_, b_, slot_):
        return pltpu.make_async_copy(v_hbm[c].at[b_, pl.ds(hg_ * G, G)],
                                     v_buf.at[slot_, c],
                                     kv_sem.at[slot_ * 4 + c * 2 + 1])

    def wq_all(c, hg_, wslot_):
        col = pl.multiple_of(hg_ * GD, GD)
        return pltpu.make_async_copy(wq_hbm[c].at[:, pl.ds(col, GD)],
                                     wq_buf.at[wslot_, c],
                                     w_sem.at[wslot_ * 4 + c * 2])

    def wo_all(c, hg_, wslot_):
        row = pl.multiple_of(hg_ * GD, GD)
        return pltpu.make_async_copy(wo_hbm[c].at[pl.ds(row, GD), :],
                                     wo_buf.at[wslot_, c],
                                     w_sem.at[wslot_ * 4 + c * 2 + 1])

    def wq_piece(c, hg_, h_, wslot_):
        col = pl.multiple_of(hg_ * GD + h_ * Dh, Dh)
        dcol = pl.multiple_of(h_ * Dh, Dh)
        return pltpu.make_async_copy(wq_hbm[c].at[:, pl.ds(col, Dh)],
                                     wq_buf.at[wslot_, c, :, pl.ds(dcol, Dh)],
                                     w_sem.at[wslot_ * 4 + c * 2])

    def wo_piece(c, hg_, h_, wslot_):
        row = pl.multiple_of(hg_ * GD + h_ * Dh, Dh)
        drow = pl.multiple_of(h_ * Dh, Dh)
        return pltpu.make_async_copy(wo_hbm[c].at[pl.ds(row, Dh), :],
                                     wo_buf.at[wslot_, c, pl.ds(drow, Dh), :],
                                     w_sem.at[wslot_ * 4 + c * 2 + 1])

    @pl.when(step == 0)
    def _():
        for c in range(2):
            x_copy(c, 0).start()
            wq_all(c, 0, 0).start()
            k_copy(c, 0, 0, 0).start()
            v_copy(c, 0, 0, 0).start()
            wo_all(c, 0, 0).start()

    @pl.when(hg == 0)
    def _():
        for c in range(2):
            x_copy(c, b).wait()

        @pl.when(b + 1 < NB)
        def _():
            for c in range(2):
                x_copy(c, b + 1).start()

    @pl.when(b == 0)
    def _():
        for c in range(2):
            wq_all(c, hg, wslot).wait()
            wo_all(c, hg, wslot).wait()

    for c in range(2):
        k_copy(c, hg, b, slot).wait()
        v_copy(c, hg, b, slot).wait()

    nxt = lax.rem(step + 1, n_steps)
    hg_n = lax.div(nxt, NB)
    b_n = lax.rem(nxt, NB)
    hg_w = lax.rem(hg + 1, NHG)

    def prefetch_kv():
        for c in range(2):
            k_copy(c, hg_n, b_n, 1 - slot).start()
            v_copy(c, hg_n, b_n, 1 - slot).start()

    def prefetch_w():
        for c in range(2):
            wq_piece(c, hg_w, b, 1 - wslot).start()
            wo_piece(c, hg_w, b, 1 - wslot).start()

    prefetch_kv()

    def qp(u):
        c, h = units[u]
        q = jnp.dot(x_buf[c, b], wq_buf[wslot, c, :, h * Dh:(h + 1) * Dh],
                    preferred_element_type=jnp.float32) * scale
        return q.astype(jnp.bfloat16)

    def qk(u, q):
        c, h = units[u]
        return lax.dot_general(q, k_buf[slot, c, h], (((1,), (1,)), ((), ())),
                               preferred_element_type=jnp.float32)

    def pv(u, s):
        c, h = units[u]
        m = jnp.max(s, axis=-1, keepdims=True)
        p = jnp.exp(s - m)
        l = jnp.sum(p, axis=-1, keepdims=True)
        o = jnp.dot(p.astype(jnp.bfloat16), v_buf[slot, c, h],
                    preferred_element_type=jnp.float32)
        o = o * pl.reciprocal(l, approx=False)
        return o.astype(jnp.bfloat16)

    def op(u, o):
        c, h = units[u]
        y = jnp.dot(o, wo_buf[wslot, c, h * Dh:(h + 1) * Dh, :],
                    preferred_element_type=jnp.float32)
        prev = acc_ref[b, :, c * D:(c + 1) * D]
        if h == 0:
            prev = jnp.where(hg == 0, jnp.zeros_like(prev), prev)
        new = prev + y
        acc_ref[b, :, c * D:(c + 1) * D] = new
        if h == G - 1:
            o_ref[0, :, c * D:(c + 1) * D] = new.astype(o_ref.dtype)

    qs, ss, os_ = {}, {}, {}
    for t in range(n + 3):
        if t == 4:
            prefetch_w()
        if t < n:
            qs[t] = qp(t)
        if 0 <= t - 1 < n:
            ss[t - 1] = qk(t - 1, qs.pop(t - 1))
        if 0 <= t - 2 < n:
            os_[t - 2] = pv(t - 2, ss.pop(t - 2))
        if 0 <= t - 3 < n:
            op(t - 3, os_.pop(t - 3))

    @pl.when(step == n_steps - 1)
    def _():
        for c in range(2):
            k_copy(c, 0, 0, 1 - slot).wait()
            v_copy(c, 0, 0, 1 - slot).wait()
            wq_all(c, 0, 1 - wslot).wait()
            wo_all(c, 0, 1 - wslot).wait()


@jax.jit
def pallas_concat_heads__mha_block_cached__mha_block_cached__near_ridge_kernel(
    A_x: jax.Array,
    A_k_cache: jax.Array,
    A_v_cache: jax.Array,
    A_wq: jax.Array,
    A_wo: jax.Array,
    B_x: jax.Array,
    B_k_cache: jax.Array,
    B_v_cache: jax.Array,
    B_wq: jax.Array,
    B_wo: jax.Array,
):
    NB, Sq, D = A_x.shape
    _, H, Sk, Dh = A_k_cache.shape
    G = NB
    NHG = H // G
    dt = A_x.dtype

    any_spec = pl.BlockSpec(memory_space=pl.ANY)
    out_spec = pl.BlockSpec(
        (1, Sq, 2 * D),
        lambda hg, b: (jnp.where(hg == NHG - 1, b, 0), 0, 0))

    kernel = functools.partial(_kernel, G=G, Dh=Dh, D=D, NB=NB, NHG=NHG)
    return pl.pallas_call(
        kernel,
        grid=(NHG, NB),
        in_specs=[any_spec] * 10,
        out_specs=out_spec,
        out_shape=jax.ShapeDtypeStruct((NB, Sq, 2 * D), dt),
        scratch_shapes=[
            pltpu.VMEM((2, NB, Sq, D), dt),
            pltpu.VMEM((2, 2, G, Sk, Dh), dt),
            pltpu.VMEM((2, 2, G, Sk, Dh), dt),
            pltpu.VMEM((2, 2, D, G * Dh), dt),
            pltpu.VMEM((2, 2, G * Dh, D), dt),
            pltpu.VMEM((NB, Sq, 2 * D), jnp.float32),
            pltpu.SemaphoreType.DMA((4,)),
            pltpu.SemaphoreType.DMA((8,)),
            pltpu.SemaphoreType.DMA((8,)),
        ],
        compiler_params=pltpu.CompilerParams(
            dimension_semantics=("arbitrary", "arbitrary"),
            vmem_limit_bytes=100 * 1024 * 1024,
        ),
    )(A_x, A_k_cache, A_v_cache, A_wq, A_wo,
      B_x, B_k_cache, B_v_cache, B_wq, B_wo)
```

```python
import functools

import jax
import jax.numpy as jnp
from jax import lax
import jax.experimental.pallas as pl
import jax.experimental.pallas.tpu as pltpu


def _kernel(ax_hbm, ak_hbm, av_hbm, awq_hbm, awo_hbm,
            bx_hbm, bk_hbm, bv_hbm, bwq_hbm, bwo_hbm,
            o_ref,
            x_buf, k_buf, v_buf, wq_buf, wo_buf, q_buf, acc_ref,
            x_sem, kv_sem, w_sem, *, G, Dh, D, NB, NHG):
    hg = pl.program_id(0)
    b = pl.program_id(1)
    step = hg * NB + b
    n_steps = NHG * NB
    slot = lax.rem(step, 3)
    gslot = lax.rem(hg, 2)
    scale = Dh ** -0.5
    GD = G * Dh

    x_hbm = (ax_hbm, bx_hbm)
    k_hbm = (ak_hbm, bk_hbm)
    v_hbm = (av_hbm, bv_hbm)
    wq_hbm = (awq_hbm, bwq_hbm)
    wo_hbm = (awo_hbm, bwo_hbm)

    units = [(c, h) for c in range(2) for h in range(G)]
    n = len(units)

    def x_copy(c):
        return pltpu.make_async_copy(x_hbm[c], x_buf.at[c], x_sem.at[c])

    def k_copy(c, hg_, b_, slot_):
        return pltpu.make_async_copy(k_hbm[c].at[b_, pl.ds(hg_ * G, G)],
                                     k_buf.at[slot_, c],
                                     kv_sem.at[slot_ * 4 + c * 2])

    def v_copy(c, hg_, b_, slot_):
        return pltpu.make_async_copy(v_hbm[c].at[b_, pl.ds(hg_ * G, G)],
                                     v_buf.at[slot_, c],
                                     kv_sem.at[slot_ * 4 + c * 2 + 1])

    def wq_all(c, hg_, wslot_):
        col = pl.multiple_of(hg_ * GD, GD)
        return pltpu.make_async_copy(wq_hbm[c].at[:, pl.ds(col, GD)],
                                     wq_buf.at[wslot_, c],
                                     w_sem.at[wslot_ * 4 + c * 2])

    def wo_all(c, hg_, wslot_):
        row = pl.multiple_of(hg_ * GD, GD)
        return pltpu.make_async_copy(wo_hbm[c].at[pl.ds(row, GD), :],
                                     wo_buf.at[wslot_, c],
                                     w_sem.at[wslot_ * 4 + c * 2 + 1])

    def wq_piece(c, hg_, h_, wslot_):
        col = pl.multiple_of(hg_ * GD + h_ * Dh, Dh)
        dcol = pl.multiple_of(h_ * Dh, Dh)
        return pltpu.make_async_copy(wq_hbm[c].at[:, pl.ds(col, Dh)],
                                     wq_buf.at[wslot_, c, :, pl.ds(dcol, Dh)],
                                     w_sem.at[wslot_ * 4 + c * 2])

    def wo_piece(c, hg_, h_, wslot_):
        row = pl.multiple_of(hg_ * GD + h_ * Dh, Dh)
        drow = pl.multiple_of(h_ * Dh, Dh)
        return pltpu.make_async_copy(wo_hbm[c].at[pl.ds(row, Dh), :],
                                     wo_buf.at[wslot_, c, pl.ds(drow, Dh), :],
                                     w_sem.at[wslot_ * 4 + c * 2 + 1])

    @pl.when(step == 0)
    def _():
        Sq = x_buf.shape[2]

        def qphase(c, lo, hi):
            def qbody(j, carry):
                bb = pl.multiple_of(j * 2, 2)
                xx = x_buf[c, pl.ds(bb, 2)].reshape(2 * Sq, D)
                q = jnp.dot(xx, wq_buf[0, c],
                            preferred_element_type=jnp.float32) * scale
                q_buf[0, c, pl.ds(bb, 2)] = q.astype(q_buf.dtype).reshape(2, Sq, GD)
                return carry
            lax.fori_loop(lo // 2, hi // 2, qbody, 0)

        x_copy(0).start()
        wq_all(0, 0, 0).start()
        x_copy(0).wait()
        wq_all(0, 0, 0).wait()
        x_copy(1).start()
        wq_all(1, 0, 0).start()
        qphase(0, 0, NB // 2)
        for c in range(2):
            k_copy(c, 0, 0, 0).start()
            v_copy(c, 0, 0, 0).start()
        for c in range(2):
            wo_all(c, 0, 0).start()
            wq_all(c, 1, 1).start()
        qphase(0, NB // 2, NB)
        x_copy(1).wait()
        wq_all(1, 0, 0).wait()
        for c in range(2):
            k_copy(c, 0, 1, 1).start()
            v_copy(c, 0, 1, 1).start()
        qphase(1, 0, NB)

    @pl.when(b == 0)
    def _():
        for c in range(2):
            wq_all(c, 0, 1 - gslot).wait()
            wo_all(c, 0, gslot).wait()

    for c in range(2):
        k_copy(c, hg, b, slot).wait()
        v_copy(c, hg, b, slot).wait()

    def prefetch_kv():
        nxt = step + 2
        hg_n = lax.div(nxt, NB)
        b_n = lax.rem(nxt, NB)
        slot_n = lax.rem(nxt, 3)
        for c in range(2):
            k_copy(c, hg_n, b_n, slot_n).start()
            v_copy(c, hg_n, b_n, slot_n).start()

    def prefetch_w():
        hg_q = lax.rem(hg + 2, NHG)
        for c in range(2):
            wq_piece(c, hg_q, b, gslot).start()
            wo_piece(c, hg + 1, b, 1 - gslot).start()

    def qp(u):
        c, h = units[u]
        q = jnp.dot(x_buf[c, b], wq_buf[1 - gslot, c, :, h * Dh:(h + 1) * Dh],
                    preferred_element_type=jnp.float32) * scale
        q_buf[1 - gslot, c, b, :, h * Dh:(h + 1) * Dh] = q.astype(q_buf.dtype)

    def qk(u):
        c, h = units[u]
        q = q_buf[gslot, c, b, :, h * Dh:(h + 1) * Dh]
        return lax.dot_general(q, k_buf[slot, c, h], (((1,), (1,)), ((), ())),
                               preferred_element_type=jnp.float32)

    def pv(u, s):
        c, h = units[u]
        m = jnp.max(s, axis=-1, keepdims=True)
        p = jnp.exp(s - m)
        l = jnp.sum(p, axis=-1, keepdims=True)
        o = jnp.dot(p.astype(jnp.bfloat16), v_buf[slot, c, h],
                    preferred_element_type=jnp.float32)
        r = pl.reciprocal(l, approx=True)
        r = r * (2.0 - l * r)
        o = o * r
        return o.astype(jnp.bfloat16)

    def op(u, o_list):
        c, h = units[u]
        nh = len(o_list)
        o = o_list[0] if nh == 1 else jnp.concatenate(o_list, axis=-1)
        y = jnp.dot(o, wo_buf[gslot, c, h * Dh:(h + nh) * Dh, :],
                    preferred_element_type=jnp.float32)
        prev = acc_ref[b, :, c * D:(c + 1) * D]
        if h == 0:
            prev = jnp.where(hg == 0, jnp.zeros_like(prev), prev)
        new = prev + y
        acc_ref[b, :, c * D:(c + 1) * D] = new
        if h + nh == G:
            o_ref[0, :, c * D:(c + 1) * D] = new.astype(o_ref.dtype)

    def body(with_q):
        ss, os_ = {}, {}
        for t in range(n + 2):
            if t == 1 and with_q:
                prefetch_kv()
            if t == 4 and with_q:
                prefetch_w()
            if t < n:
                ss[t] = qk(t)
                if with_q:
                    qp(t)
            if 0 <= t - 1 < n:
                os_[t - 1] = pv(t - 1, ss.pop(t - 1))
            u = t - 2
            if 0 <= u < n - 2 and u % 2 == 1:
                op(u - 1, [os_.pop(u - 1), os_.pop(u)])
            elif u >= n - 2:
                op(u, [os_.pop(u)])

    @pl.when(hg < NHG - 1)
    def _():
        body(True)

    @pl.when(hg == NHG - 1)
    def _():
        pl.when(step + 2 < n_steps)(prefetch_kv)
        body(False)


@jax.jit
def pallas_concat_heads__mha_block_cached__mha_block_cached__near_ridge_kernel(
    A_x: jax.Array,
    A_k_cache: jax.Array,
    A_v_cache: jax.Array,
    A_wq: jax.Array,
    A_wo: jax.Array,
    B_x: jax.Array,
    B_k_cache: jax.Array,
    B_v_cache: jax.Array,
    B_wq: jax.Array,
    B_wo: jax.Array,
):
    NB, Sq, D = A_x.shape
    _, H, Sk, Dh = A_k_cache.shape
    G = NB
    NHG = H // G
    dt = A_x.dtype

    any_spec = pl.BlockSpec(memory_space=pl.ANY)
    out_spec = pl.BlockSpec(
        (1, Sq, 2 * D),
        lambda hg, b: (jnp.where(hg == NHG - 1, b, 0), 0, 0))

    kernel = functools.partial(_kernel, G=G, Dh=Dh, D=D, NB=NB, NHG=NHG)
    return pl.pallas_call(
        kernel,
        grid=(NHG, NB),
        in_specs=[any_spec] * 10,
        out_specs=out_spec,
        out_shape=jax.ShapeDtypeStruct((NB, Sq, 2 * D), dt),
        scratch_shapes=[
            pltpu.VMEM((2, NB, Sq, D), dt),
            pltpu.VMEM((3, 2, G, Sk, Dh), dt),
            pltpu.VMEM((3, 2, G, Sk, Dh), dt),
            pltpu.VMEM((2, 2, D, G * Dh), dt),
            pltpu.VMEM((2, 2, G * Dh, D), dt),
            pltpu.VMEM((2, 2, NB, Sq, G * Dh), dt),
            pltpu.VMEM((NB, Sq, 2 * D), jnp.float32),
            pltpu.SemaphoreType.DMA((2,)),
            pltpu.SemaphoreType.DMA((12,)),
            pltpu.SemaphoreType.DMA((8,)),
        ],
        compiler_params=pltpu.CompilerParams(
            dimension_semantics=("arbitrary", "arbitrary"),
            vmem_limit_bytes=100 * 1024 * 1024,
        ),
    )(A_x, A_k_cache, A_v_cache, A_wq, A_wo,
      B_x, B_k_cache, B_v_cache, B_wq, B_wo)
```

```python
import functools

import jax
import jax.numpy as jnp
from jax import lax
import jax.experimental.pallas as pl
import jax.experimental.pallas.tpu as pltpu


def _kernel(ax_hbm, ak_hbm, av_hbm, awq_hbm, awo_hbm,
            bx_hbm, bk_hbm, bv_hbm, bwq_hbm, bwo_hbm,
            o_ref,
            x_buf, k_buf, v_buf, wq_buf, wo_buf, q_buf, acc_ref,
            x_sem, kv_sem, w_sem, *, G, Dh, D, NB, NHG):
    hg = pl.program_id(0)
    b = pl.program_id(1)
    step = hg * NB + b
    n_steps = NHG * NB
    slot = lax.rem(step, 3)
    gslot = lax.rem(hg, 2)
    scale = Dh ** -0.5
    GD = G * Dh

    x_hbm = (ax_hbm, bx_hbm)
    k_hbm = (ak_hbm, bk_hbm)
    v_hbm = (av_hbm, bv_hbm)
    wq_hbm = (awq_hbm, bwq_hbm)
    wo_hbm = (awo_hbm, bwo_hbm)

    units = [(c, h) for c in range(2) for h in range(G)]
    n = len(units)

    def x_copy(c):
        return pltpu.make_async_copy(x_hbm[c], x_buf.at[c], x_sem.at[c])

    def k_copy(c, hg_, b_, slot_):
        return pltpu.make_async_copy(k_hbm[c].at[b_, pl.ds(hg_ * G, G)],
                                     k_buf.at[slot_, c],
                                     kv_sem.at[slot_ * 4 + c * 2])

    def v_copy(c, hg_, b_, slot_):
        return pltpu.make_async_copy(v_hbm[c].at[b_, pl.ds(hg_ * G, G)],
                                     v_buf.at[slot_, c],
                                     kv_sem.at[slot_ * 4 + c * 2 + 1])

    def wq_all(c, hg_, wslot_):
        col = pl.multiple_of(hg_ * GD, GD)
        return pltpu.make_async_copy(wq_hbm[c].at[:, pl.ds(col, GD)],
                                     wq_buf.at[wslot_, c],
                                     w_sem.at[wslot_ * 4 + c * 2])

    def wo_all(c, hg_, wslot_):
        row = pl.multiple_of(hg_ * GD, GD)
        return pltpu.make_async_copy(wo_hbm[c].at[pl.ds(row, GD), :],
                                     wo_buf.at[wslot_, c],
                                     w_sem.at[wslot_ * 4 + c * 2 + 1])

    def wq_piece(c, hg_, h_, wslot_):
        col = pl.multiple_of(hg_ * GD + h_ * Dh, Dh)
        dcol = pl.multiple_of(h_ * Dh, Dh)
        return pltpu.make_async_copy(wq_hbm[c].at[:, pl.ds(col, Dh)],
                                     wq_buf.at[wslot_, c, :, pl.ds(dcol, Dh)],
                                     w_sem.at[wslot_ * 4 + c * 2])

    def wo_piece(c, hg_, h_, wslot_):
        row = pl.multiple_of(hg_ * GD + h_ * Dh, Dh)
        drow = pl.multiple_of(h_ * Dh, Dh)
        return pltpu.make_async_copy(wo_hbm[c].at[pl.ds(row, Dh), :],
                                     wo_buf.at[wslot_, c, pl.ds(drow, Dh), :],
                                     w_sem.at[wslot_ * 4 + c * 2 + 1])

    @pl.when(step == 0)
    def _():
        Sq = x_buf.shape[2]

        def qphase(c, lo, hi):
            def qbody(j, carry):
                bb = pl.multiple_of(j * 2, 2)
                xx = x_buf[c, pl.ds(bb, 2)].reshape(2 * Sq, D)
                q = jnp.dot(xx, wq_buf[0, c],
                            preferred_element_type=jnp.float32) * scale
                q_buf[0, c, pl.ds(bb, 2)] = q.astype(q_buf.dtype).reshape(2, Sq, GD)
                return carry
            lax.fori_loop(lo // 2, hi // 2, qbody, 0)

        x_copy(0).start()
        wq_all(0, 0, 0).start()
        x_copy(0).wait()
        wq_all(0, 0, 0).wait()
        x_copy(1).start()
        wq_all(1, 0, 0).start()
        qphase(0, 0, NB // 2)
        for c in range(2):
            k_copy(c, 0, 0, 0).start()
            v_copy(c, 0, 0, 0).start()
        for c in range(2):
            wo_all(c, 0, 0).start()
            wq_all(c, 1, 1).start()
        qphase(0, NB // 2, NB)
        x_copy(1).wait()
        wq_all(1, 0, 0).wait()
        for c in range(2):
            k_copy(c, 0, 1, 1).start()
            v_copy(c, 0, 1, 1).start()
        qphase(1, 0, NB)

    @pl.when(b == 0)
    def _():
        for c in range(2):
            wq_all(c, 0, 1 - gslot).wait()
            wo_all(c, 0, gslot).wait()

    for c in range(2):
        k_copy(c, hg, b, slot).wait()
        v_copy(c, hg, b, slot).wait()

    def prefetch_kv():
        nxt = step + 2
        hg_n = lax.div(nxt, NB)
        b_n = lax.rem(nxt, NB)
        slot_n = lax.rem(nxt, 3)
        for c in range(2):
            k_copy(c, hg_n, b_n, slot_n).start()
            v_copy(c, hg_n, b_n, slot_n).start()

    def prefetch_w():
        hg_q = lax.rem(hg + 2, NHG)
        for c in range(2):
            wq_piece(c, hg_q, b, gslot).start()
            wo_piece(c, hg + 1, b, 1 - gslot).start()

    def qp(u):
        c, h = units[u]
        q = jnp.dot(x_buf[c, b], wq_buf[1 - gslot, c, :, h * Dh:(h + 1) * Dh],
                    preferred_element_type=jnp.float32) * scale
        q_buf[1 - gslot, c, b, :, h * Dh:(h + 1) * Dh] = q.astype(q_buf.dtype)

    def qk(u):
        c, h = units[u]
        q = q_buf[gslot, c, b, :, h * Dh:(h + 1) * Dh]
        return lax.dot_general(q, k_buf[slot, c, h], (((1,), (1,)), ((), ())),
                               preferred_element_type=jnp.float32)

    def pv(u, s):
        c, h = units[u]
        m = jnp.max(s, axis=-1, keepdims=True)
        p = jnp.exp(s - m)
        l = jnp.sum(p, axis=-1, keepdims=True)
        o = jnp.dot(p.astype(jnp.bfloat16), v_buf[slot, c, h],
                    preferred_element_type=jnp.float32)
        r = pl.reciprocal(l, approx=True)
        r = r * (2.0 - l * r)
        o = o * r
        return o.astype(jnp.bfloat16)

    def op(u, o_list):
        c, h = units[u]
        nh = len(o_list)
        o = o_list[0] if nh == 1 else jnp.concatenate(o_list, axis=-1)
        y = jnp.dot(o, wo_buf[gslot, c, h * Dh:(h + nh) * Dh, :],
                    preferred_element_type=jnp.float32)
        prev = acc_ref[b, :, c * D:(c + 1) * D]
        if h == 0:
            prev = jnp.where(hg == 0, jnp.zeros_like(prev), prev)
        new = prev + y
        acc_ref[b, :, c * D:(c + 1) * D] = new
        if h + nh == G:
            o_ref[0, :, c * D:(c + 1) * D] = new.astype(o_ref.dtype)

    def body(with_q):
        ss, os_ = {}, {}
        ss[0] = qk(0)
        ss[1] = qk(1)
        for t in range(n + 1):
            if t == 1 and with_q:
                prefetch_kv()
            if t == 4 and with_q:
                prefetch_w()
            if t < n:
                if with_q:
                    qp(t)
                os_[t] = pv(t, ss.pop(t))
            u = t - 1
            if 0 <= u < n - 2 and u % 2 == 1:
                op(u - 1, [os_.pop(u - 1), os_.pop(u)])
            elif u >= n - 2:
                op(u, [os_.pop(u)])
            if t + 2 < n:
                ss[t + 2] = qk(t + 2)

    @pl.when(hg < NHG - 1)
    def _():
        body(True)

    @pl.when(hg == NHG - 1)
    def _():
        pl.when(step + 2 < n_steps)(prefetch_kv)
        body(False)


@jax.jit
def pallas_concat_heads__mha_block_cached__mha_block_cached__near_ridge_kernel(
    A_x: jax.Array,
    A_k_cache: jax.Array,
    A_v_cache: jax.Array,
    A_wq: jax.Array,
    A_wo: jax.Array,
    B_x: jax.Array,
    B_k_cache: jax.Array,
    B_v_cache: jax.Array,
    B_wq: jax.Array,
    B_wo: jax.Array,
):
    NB, Sq, D = A_x.shape
    _, H, Sk, Dh = A_k_cache.shape
    G = NB
    NHG = H // G
    dt = A_x.dtype

    any_spec = pl.BlockSpec(memory_space=pl.ANY)
    out_spec = pl.BlockSpec(
        (1, Sq, 2 * D),
        lambda hg, b: (jnp.where(hg == NHG - 1, b, 0), 0, 0))

    kernel = functools.partial(_kernel, G=G, Dh=Dh, D=D, NB=NB, NHG=NHG)
    return pl.pallas_call(
        kernel,
        grid=(NHG, NB),
        in_specs=[any_spec] * 10,
        out_specs=out_spec,
        out_shape=jax.ShapeDtypeStruct((NB, Sq, 2 * D), dt),
        scratch_shapes=[
            pltpu.VMEM((2, NB, Sq, D), dt),
            pltpu.VMEM((3, 2, G, Sk, Dh), dt),
            pltpu.VMEM((3, 2, G, Sk, Dh), dt),
            pltpu.VMEM((2, 2, D, G * Dh), dt),
            pltpu.VMEM((2, 2, G * Dh, D), dt),
            pltpu.VMEM((2, 2, NB, Sq, G * Dh), dt),
            pltpu.VMEM((NB, Sq, 2 * D), jnp.float32),
            pltpu.SemaphoreType.DMA((2,)),
            pltpu.SemaphoreType.DMA((12,)),
            pltpu.SemaphoreType.DMA((8,)),
        ],
        compiler_params=pltpu.CompilerParams(
            dimension_semantics=("arbitrary", "arbitrary"),
            vmem_limit_bytes=100 * 1024 * 1024,
        ),
    )(A_x, A_k_cache, A_v_cache, A_wq, A_wo,
      B_x, B_k_cache, B_v_cache, B_wq, B_wo)
```
